```python
import jax
import jax.numpy as jnp

def _softmax(x, axis=-1):
    return jax.nn.softmax(x, axis=axis)

def _gelu(x):
    return jax.nn.gelu(x, approximate=True)

def _silu(x):
    return jax.nn.silu(x)

def _sigmoid(x):
    return jax.nn.sigmoid(x)

def _layernorm(x, axis=-1, eps=1e-05):
    m = jnp.mean(x, axis=axis, keepdims=True)
    v = jnp.var(x, axis=axis, keepdims=True)
    return (x - m) / jnp.sqrt(v + eps)

def _scatter_add(tgt, idx, src, axis=0):
    return tgt.at[idx].add(src)

def _segment_sum(src, seg, n):
    return jax.ops.segment_sum(src, seg, n)

class _Rng:

    def __init__(self, key):
        self._k = key

    def _next(self):
        self._k, sub = jax.random.split(self._k)
        return sub

    def normal(self, shape):
        return jax.random.normal(self._next(), shape, dtype=jnp.bfloat16)

    def randint(self, lo, hi, shape):
        return jax.random.randint(self._next(), shape, lo, hi, dtype=jnp.int32)

    def uniform(self, shape, lo=0.0, hi=1.0):
        return jax.random.uniform(self._next(), shape, jnp.bfloat16, lo, hi)

    def permutation(self, n):
        return jax.random.permutation(self._next(), n)
kernel_name = 'adaLN_cond__sliding_local_dilated__mixer_s_mlp__prompt'

def setup_inputs():
    _rng = _Rng(jax.random.key(int.from_bytes(__import__("os").urandom(4), "little")))
    _w = lambda a: (lambda t: t.astype(jnp.bfloat16) if jnp.issubdtype(t.dtype, jnp.floating) else t)(jnp.asarray(a))

    def _A_setup():
        B, S, D = (1, 2048, 1024)
        return {'x': _w((lambda *s: _rng.normal(s) * 0.05)(B, S, D)), 'wqkv': _w((lambda *s: _rng.normal(s) * 0.05)(D, 3 * D)), 'wo': _w((lambda *s: _rng.normal(s) * 0.05)(D, D))}
    _A_in = _A_setup()

    def _B_setup():
        B, S, D, F = (1, 2048, 1024, 3584)
        return {'x': _w((lambda *s: _rng.normal(s) * 0.05)(B, S, D)), 'w1': _w((lambda *s: _rng.normal(s) * 0.05)(D, D) * D ** (-0.5)), 'w2': _w((lambda *s: _rng.normal(s) * 0.05)(D, D) * D ** (-0.5)), 'w3': _w((lambda *s: _rng.normal(s) * 0.05)(D, F) * D ** (-0.5)), 'w4': _w((lambda *s: _rng.normal(s) * 0.05)(F, D) * F ** (-0.5))}
    _B_in = _B_setup()
    return {'A_x': _A_in['x'], 'A_wqkv': _A_in['wqkv'], 'A_wo': _A_in['wo'], 'B_x': _B_in['x'], 'B_w1': _B_in['w1'], 'B_w2': _B_in['w2'], 'B_w3': _B_in['w3'], 'B_w4': _B_in['w4'], 'c': _w((lambda *s: _rng.normal(s) * 0.05)(1, 1024)), 'w_mod': _w((lambda *s: _rng.normal(s) * 0.05)(1024, 6 * 1024) * 1024 ** (-0.5))}

def reference(A_x, A_wqkv, A_wo, B_x, B_w1, B_w2, B_w3, B_w4, c, w_mod):

    def _A_ref(x, wqkv, wo):
        B, S, D = x.shape
        H = 32
        Dh = D // H
        W, dil = (8, 2)
        qkv = (lambda x, *d: x.transpose(*d))((x @ wqkv).reshape(B, S, 3, H, Dh), 2, 0, 3, 1, 4)
        q, k, v = (qkv[0], qkv[1], qkv[2])
        scale = Dh ** (-0.5)
        pos = jnp.arange(S)
        off = jnp.arange(W) * dil
        idx = pos[:, None] - off[None, :]
        mask = idx >= 0
        idx_c = jnp.where(mask, idx, 0).reshape(-1)
        kg = k[:, :, idx_c, :].reshape(B, H, S, W, Dh)
        vg = v[:, :, idx_c, :].reshape(B, H, S, W, Dh)
        logits = jnp.einsum('bhsd,bhswd->bhsw', q, kg) * scale
        logits = jnp.where(mask[None, None, :, :], logits, -1000000000.0)
        attn = _softmax(logits, axis=-1)
        o = jnp.einsum('bhsw,bhswd->bhsd', attn, vg)
        return (lambda x, *d: x.transpose(*d))(o, 0, 2, 1, 3).reshape(B, S, D) @ wo

    def _B_ref(x, w1, w2, w3, w4):
        B, S, D = x.shape
        h = _gelu(_layernorm(x, axis=-1) @ w1)
        c = D // 4
        g0 = jnp.pad(h[:, :, 0 * c:1 * c], ((0, 0), (1, 0), (0, 0)))[:, :S, :]
        g1 = jnp.pad(h[:, :, 1 * c:2 * c], ((0, 0), (0, 1), (0, 0)))[:, 1:, :]
        g2 = jnp.pad(h[:, :, 2 * c:3 * c], ((0, 0), (2, 0), (0, 0)))[:, :S, :]
        g3 = jnp.pad(h[:, :, 3 * c:], ((0, 0), (0, 2), (0, 0)))[:, 2:, :]
        hs = jnp.concatenate([g0, g1, g2, g3], axis=-1) @ w2
        x1 = x + hs
        h2 = _gelu(_layernorm(x1, axis=-1) @ w3) @ w4
        return x1 + h2
    x = A_x
    mod = (_silu(c) @ w_mod).reshape(c.shape[0], 6, 1, -1)
    sa, ca, ga, sb, cb, gb = (mod[:, 0].copy(), mod[:, 1].copy(), mod[:, 2].copy(), mod[:, 3].copy(), mod[:, 4].copy(), mod[:, 5].copy())
    h = _layernorm(x, axis=-1) * (1 + ca) + sa
    x = x + ga * _A_ref(h, A_wqkv, A_wo)
    h = _layernorm(x, axis=-1) * (1 + cb) + sb
    x = x + gb * _B_ref(h, B_w1, B_w2, B_w3, B_w4)
    return x
```

```python
import jax
import jax.numpy as jnp
from jax import lax
import jax.experimental.pallas as pl
import jax.experimental.pallas.tpu as pltpu

S, D, F = 2048, 1024, 3584
T = 256
NT = S // T
LAG = 2
PAD = 16
W, DIL, DH = 8, 2, 32
FC = 512
f32, bf16 = jnp.float32, jnp.bfloat16


def _ln(x):
    m = jnp.mean(x, axis=-1, keepdims=True)
    d = x - m
    v = jnp.mean(d * d, axis=-1, keepdims=True)
    return d * lax.rsqrt(v + 1e-5)


def _gelu(x):
    u = x * (0.7978845608028654 + (0.7978845608028654 * 0.044715) * (x * x))
    hx = 0.5 * x
    return hx + hx * jnp.tanh(u)


def _dot(a, b):
    return jnp.dot(a, b, preferred_element_type=f32)


def _interleave(*gens):
    gens = list(gens)
    while gens:
        for g in list(gens):
            try:
                next(g)
            except StopIteration:
                gens.remove(g)


def _kernel(x_ref, c_ref, wmod_h, wqkv_h, wo_h, w1_h, w2_h, w3_h, w4_h, o_ref,
            wmod, wqkv, wo, w1, w2, w3, w4, mod, kb, vb, ob, xa, hb, gs, ub, sems):
    i = pl.program_id(0)
    cps = [
        pltpu.make_async_copy(wmod_h.at[:, 0:2 * D], wmod.at[:, 0:2 * D], sems.at[0]),
        pltpu.make_async_copy(wqkv_h, wqkv, sems.at[1]),
        pltpu.make_async_copy(wmod_h.at[:, 2 * D:], wmod.at[:, 2 * D:], sems.at[2]),
        pltpu.make_async_copy(wo_h, wo, sems.at[3]),
        pltpu.make_async_copy(w1_h, w1, sems.at[4]),
        pltpu.make_async_copy(w2_h, w2, sems.at[5]),
        pltpu.make_async_copy(w3_h, w3, sems.at[6]),
        pltpu.make_async_copy(w4_h, w4, sems.at[7]),
    ]

    def mrow(j):
        return mod[0:1, j * D:(j + 1) * D]

    def stage_a(t):
        r0 = pl.multiple_of(t * T, T)
        x = x_ref[...].astype(f32)
        h = (_ln(x) * (1.0 + mrow(1)) + mrow(0)).astype(bf16)
        yield
        q = _dot(h, wqkv[:, 0:D]) * (DH ** -0.5)
        kb[PAD:, :] = _dot(h, wqkv[:, D:2 * D])
        vb[PAD:, :] = _dot(h, wqkv[:, 2 * D:])
        yield
        li = lax.broadcasted_iota(jnp.int32, (128, 128), 0) // DH
        lj = lax.broadcasted_iota(jnp.int32, (128, 128), 1) // DH
        ones = (li == lj).astype(bf16)
        pos = r0 + lax.broadcasted_iota(jnp.int32, (T, 128), 0)
        for g in range(D // 128):
            cs = slice(g * 128, (g + 1) * 128)
            qg = q[:, cs]
            ls = []
            for w in range(W):
                p = (qg * kb[PAD - DIL * w:PAD - DIL * w + T, cs]).astype(bf16)
                l = _dot(p, ones)
                if w:
                    l = jnp.where(pos >= DIL * w, l, -1e9)
                ls.append(l)
            m = ls[0]
            for l in ls[1:]:
                m = jnp.maximum(m, l)
            den = None
            for w in range(W):
                e = jnp.exp(ls[w] - m)
                ev = e * vb[PAD - DIL * w:PAD - DIL * w + T, cs]
                den = e if den is None else den + e
                acc = ev if w == 0 else acc + ev
            ob[:, cs] = (acc / den).astype(bf16)
            yield
        kb[0:PAD, :] = kb[T:T + PAD, :]
        vb[0:PAD, :] = vb[T:T + PAD, :]
        x1 = x_ref[...].astype(f32) + mrow(2) * _dot(ob[...], wo[...])
        xa[pl.ds(r0, T), :] = x1
        h2 = _ln(x1) * (1.0 + mrow(4)) + mrow(3)
        hb[pl.ds(r0, T), :] = h2
        yield
        g1 = _gelu(_dot(_ln(h2).astype(bf16), w1[...]))
        gs[pl.ds(r0 + 8, T), :] = g1

    def stage_b(t):
        r0 = pl.multiple_of(t * T, T)
        c = D // 4
        win = gs[pl.ds(r0, T + 16), :]
        gsh = jnp.concatenate([
            win[7:7 + T, 0:c], win[9:9 + T, c:2 * c],
            win[6:6 + T, 2 * c:3 * c], win[10:10 + T, 3 * c:]], axis=1).astype(bf16)
        x1 = hb[pl.ds(r0, T), :] + _dot(gsh, w2[...])
        hb[pl.ds(r0, T), :] = x1
        l = _ln(x1).astype(bf16)
        yield
        for j in range(F // FC):
            ub[:, j * FC:(j + 1) * FC] = _gelu(_dot(l, w3[:, j * FC:(j + 1) * FC])).astype(bf16)
            yield
        for j in range(2):
            cs = slice(j * 512, (j + 1) * 512)
            h2 = _dot(ub[...], w4[:, cs])
            o_ref[:, cs] = (xa[pl.ds(r0, T), cs]
                            + mod[0:1, 5 * D + j * 512:5 * D + (j + 1) * 512]
                            * (hb[pl.ds(r0, T), cs] + h2)).astype(o_ref.dtype)
            yield

    @pl.when(i == 0)
    def _():
        for cp in cps:
            cp.start()
        kb[0:PAD, :] = jnp.zeros((PAD, D), f32)
        vb[0:PAD, :] = jnp.zeros((PAD, D), f32)
        gs[0:8, :] = jnp.zeros((8, D), f32)
        gs[S + 8:, :] = jnp.zeros((8, D), f32)
        cv = c_ref[...].astype(f32)
        sc = jnp.broadcast_to(cv * jax.nn.sigmoid(cv), (8, D)).astype(bf16)
        cps[0].wait()
        mod[:, 0:2 * D] = _dot(sc, wmod[:, 0:2 * D])
        a = stage_a(i)
        next(a)
        cps[1].wait()
        for _ in range(9):
            next(a)
        cps[2].wait()
        mod[:, 2 * D:] = _dot(sc, wmod[:, 2 * D:])
        cps[3].wait()
        cps[4].wait()
        _interleave(a)

    @pl.when((i > 0) & (i < LAG))
    def _():
        _interleave(stage_a(i))

    @pl.when(i == LAG)
    def _():
        for cp in cps[5:]:
            cp.wait()

    @pl.when((i >= LAG) & (i < NT))
    def _():
        _interleave(stage_b(i - LAG), stage_a(i))

    @pl.when(i >= NT)
    def _():
        _interleave(stage_b(i - LAG))


@jax.jit
def pallas_adaLN_cond__sliding_local_dilated__mixer_s_mlp__prompt_kernel(
        A_x, A_wqkv, A_wo, B_x, B_w1, B_w2, B_w3, B_w4, c, w_mod):
    any_spec = pl.BlockSpec(memory_space=pl.ANY)
    ws = (w_mod, A_wqkv, A_wo, B_w1, B_w2, B_w3, B_w4)
    out = pl.pallas_call(
        _kernel,
        grid=(NT + LAG,),
        in_specs=[pl.BlockSpec((T, D), lambda i: (jnp.minimum(i, NT - 1), 0)),
                  pl.BlockSpec((1, D), lambda i: (0, 0))] + [any_spec] * 7,
        out_specs=pl.BlockSpec((T, D), lambda i: (jnp.maximum(i - LAG, 0), 0)),
        out_shape=jax.ShapeDtypeStruct((S, D), A_x.dtype),
        scratch_shapes=[pltpu.VMEM(w.shape, w.dtype) for w in ws] + [
            pltpu.VMEM((8, 6 * D), f32),
            pltpu.VMEM((T + PAD, D), f32), pltpu.VMEM((T + PAD, D), f32),
            pltpu.VMEM((T, D), bf16),
            pltpu.VMEM((S, D), f32), pltpu.VMEM((S, D), f32),
            pltpu.VMEM((S + 16, D), f32),
            pltpu.VMEM((T, F), bf16),
            pltpu.SemaphoreType.DMA((8,)),
        ],
        compiler_params=pltpu.CompilerParams(
            dimension_semantics=("arbitrary",),
            vmem_limit_bytes=110 * 1024 * 1024),
    )(A_x.reshape(S, D), c, *ws)
    return out.reshape(A_x.shape)
```

```python
import jax
import jax.numpy as jnp
from jax import lax
import jax.experimental.pallas as pl
import jax.experimental.pallas.tpu as pltpu

S, D, F = 2048, 1024, 3584
T = 256
NT = S // T
LAG = 2
PAD = 16
W, DIL, DH = 8, 2, 32
FC = 512
U = 2
f32, bf16 = jnp.float32, jnp.bfloat16


def _ln(x):
    m = jnp.mean(x, axis=-1, keepdims=True)
    d = x - m
    v = jnp.mean(d * d, axis=-1, keepdims=True)
    return d * lax.rsqrt(v + 1e-5)


def _gelu(x):
    u = x * (0.7978845608028654 + (0.7978845608028654 * 0.044715) * (x * x))
    hx = 0.5 * x
    return hx + hx * jnp.tanh(u)


def _dot(a, b):
    return jnp.dot(a, b, preferred_element_type=f32)


def _interleave(*gens):
    gens = list(gens)
    while gens:
        for g in list(gens):
            try:
                next(g)
            except StopIteration:
                gens.remove(g)


def _kernel(x_ref, c_ref, wmod_h, wqkv_h, wo_h, w1_h, w2_h, w3_h, w4_h, o_ref,
            wmod, wqkv, wo, w1, w2, w3, w4, mod, kb, vb, ob, xa, hb, gs, ub, qb, scb, sems):
    i = pl.program_id(0)
    cps = [
        pltpu.make_async_copy(wmod_h.at[:, 0:2 * D], wmod.at[:, 0:2 * D], sems.at[0]),
        pltpu.make_async_copy(wqkv_h, wqkv, sems.at[1]),
        pltpu.make_async_copy(wmod_h.at[:, 2 * D:], wmod.at[:, 2 * D:], sems.at[2]),
        pltpu.make_async_copy(wo_h, wo, sems.at[3]),
        pltpu.make_async_copy(w1_h, w1, sems.at[4]),
        pltpu.make_async_copy(w2_h, w2, sems.at[5]),
        pltpu.make_async_copy(w3_h, w3, sems.at[6]),
        pltpu.make_async_copy(w4_h, w4, sems.at[7]),
    ]

    def mrow(j):
        return mod[0:1, j * D:(j + 1) * D]

    def qkv():
        x = x_ref[...].astype(f32)
        h = (_ln(x) * (1.0 + mrow(1)) + mrow(0)).astype(bf16)
        qb[...] = _dot(h, wqkv[:, 0:D]) * (DH ** -0.5)
        kb[PAD:, :] = _dot(h, wqkv[:, D:2 * D])
        vb[PAD:, :] = _dot(h, wqkv[:, 2 * D:])

    def attn(t, g):
        r0 = t * T
        li = lax.broadcasted_iota(jnp.int32, (128, 128), 0) // DH
        lj = lax.broadcasted_iota(jnp.int32, (128, 128), 1) // DH
        ones = (li == lj).astype(bf16)
        pos = r0 + lax.broadcasted_iota(jnp.int32, (T, 128), 0)
        if True:
            cs = pl.ds(pl.multiple_of(g * 128, 128), 128)
            qg = qb[:, cs]
            ls = []
            for w in range(W):
                p = (qg * kb[PAD - DIL * w:PAD - DIL * w + T, cs]).astype(bf16)
                l = _dot(p, ones)
                if w:
                    l = jnp.where(pos >= DIL * w, l, -1e9)
                ls.append(l)
            m = ls[0]
            for l in ls[1:]:
                m = jnp.maximum(m, l)
            den = None
            for w in range(W):
                e = jnp.exp(ls[w] - m)
                ev = e * vb[PAD - DIL * w:PAD - DIL * w + T, cs]
                den = e if den is None else den + e
                acc = ev if w == 0 else acc + ev
            ob[:, cs] = (acc / den).astype(bf16)

    def a_back(t):
        r0 = pl.multiple_of(t * T, T)
        kb[0:PAD, :] = kb[T:T + PAD, :]
        vb[0:PAD, :] = vb[T:T + PAD, :]
        x1 = x_ref[...].astype(f32) + mrow(2) * _dot(ob[...], wo[...])
        xa[pl.ds(r0, T), :] = x1
        h2 = _ln(x1) * (1.0 + mrow(4)) + mrow(3)
        hb[pl.ds(r0, T), :] = h2
        g1 = _gelu(_dot(_ln(h2).astype(bf16), w1[...]))
        gs[pl.ds(r0 + 8, T), :] = g1

    def b_front(t):
        r0 = pl.multiple_of(t * T, T)
        c = D // 4
        win = gs[pl.ds(r0, T + 16), :]
        gsh = jnp.concatenate([
            win[7:7 + T, 0:c], win[9:9 + T, c:2 * c],
            win[6:6 + T, 2 * c:3 * c], win[10:10 + T, 3 * c:]], axis=1).astype(bf16)
        x1 = hb[pl.ds(r0, T), :] + _dot(gsh, w2[...])
        hb[pl.ds(r0, T), :] = x1
        l = _ln(x1).astype(bf16)
        for j in range(F // FC):
            ub[:, j * FC:(j + 1) * FC] = _gelu(_dot(l, w3[:, j * FC:(j + 1) * FC])).astype(bf16)

    def w4_chunk(t, g):
        r0 = pl.multiple_of(t * T, T)
        cs = pl.ds(pl.multiple_of(g * 128, 128), 128)
        gb = mod[0:1, pl.ds(pl.multiple_of(5 * D + g * 128, 128), 128)]
        h2 = _dot(ub[...], w4[:, cs])
        o_ref[:, cs] = (xa[pl.ds(r0, T), cs] + gb * (hb[pl.ds(r0, T), cs] + h2)).astype(o_ref.dtype)

    def loop(*fns):
        def body(g, carry):
            for u in range(U):
                for fn, t in fns:
                    fn(t, g * U + u)
            return carry
        lax.fori_loop(0, D // 128 // U, body, 0)

    @pl.when(i == 0)
    def _():
        for cp in cps:
            cp.start()
        kb[0:PAD, :] = jnp.zeros((PAD, D), f32)
        vb[0:PAD, :] = jnp.zeros((PAD, D), f32)
        gs[0:8, :] = jnp.zeros((8, D), f32)
        gs[S + 8:, :] = jnp.zeros((8, D), f32)
        cv = c_ref[...].astype(f32)
        sc = jnp.broadcast_to(cv * jax.nn.sigmoid(cv), (16, D)).astype(bf16)
        cps[0].wait()
        mod[:, 0:2 * D] = _dot(sc, wmod[:, 0:2 * D])
        scb[...] = sc
        cps[1].wait()

    pl.when(i < NT)(qkv)
    pl.when(i < LAG)(lambda: loop((attn, i)))
    pl.when((i >= LAG) & (i < NT))(lambda: loop((attn, i), (w4_chunk, i - LAG)))
    pl.when(i >= NT)(lambda: loop((w4_chunk, i - LAG)))

    @pl.when(i == 0)
    def _():
        for cp in cps[2:5]:
            cp.wait()

        def body(j, carry):
            cs = pl.ds(pl.multiple_of(2 * D + j * 512, 512), 512)
            mod[:, cs] = _dot(scb[...], wmod[:, cs])
            return carry
        lax.fori_loop(0, 8, body, 0)

    pl.when(i < NT)(lambda: a_back(i))

    @pl.when(i == 1)
    def _():
        for cp in cps[5:7]:
            cp.wait()

    pl.when(i == LAG - 1)(cps[7].wait)
    pl.when((i >= 1) & (i <= NT))(lambda: b_front(i - 1))


@jax.jit
def pallas_adaLN_cond__sliding_local_dilated__mixer_s_mlp__prompt_kernel(
        A_x, A_wqkv, A_wo, B_x, B_w1, B_w2, B_w3, B_w4, c, w_mod):
    any_spec = pl.BlockSpec(memory_space=pl.ANY)
    ws = (w_mod, A_wqkv, A_wo, B_w1, B_w2, B_w3, B_w4)
    out = pl.pallas_call(
        _kernel,
        grid=(NT + LAG,),
        in_specs=[pl.BlockSpec((T, D), lambda i: (jnp.minimum(i, NT - 1), 0)),
                  pl.BlockSpec((1, D), lambda i: (0, 0))] + [any_spec] * 7,
        out_specs=pl.BlockSpec((T, D), lambda i: (jnp.maximum(i - LAG, 0), 0)),
        out_shape=jax.ShapeDtypeStruct((S, D), A_x.dtype),
        scratch_shapes=[pltpu.VMEM(w.shape, w.dtype) for w in ws] + [
            pltpu.VMEM((16, 6 * D), f32),
            pltpu.VMEM((T + PAD, D), f32), pltpu.VMEM((T + PAD, D), f32),
            pltpu.VMEM((T, D), bf16),
            pltpu.VMEM((S, D), f32), pltpu.VMEM((S, D), f32),
            pltpu.VMEM((S + 16, D), f32),
            pltpu.VMEM((T, F), bf16),
            pltpu.VMEM((T, D), f32),
            pltpu.VMEM((16, D), bf16),
            pltpu.SemaphoreType.DMA((8,)),
        ],
        compiler_params=pltpu.CompilerParams(
            dimension_semantics=("arbitrary",),
            vmem_limit_bytes=110 * 1024 * 1024),
    )(A_x.reshape(S, D), c, *ws)
    return out.reshape(A_x.shape)
```

```python
import jax
import jax.numpy as jnp
from jax import lax
import jax.experimental.pallas as pl
import jax.experimental.pallas.tpu as pltpu

S, D, F = 2048, 1024, 3584
T = 256
NT = S // T
LAG = 2
PAD = 16
W, DIL, DH = 8, 2, 32
FC = 512
R = T // 8
f32, bf16 = jnp.float32, jnp.bfloat16


def _ln(x):
    m = jnp.mean(x, axis=-1, keepdims=True)
    d = x - m
    v = jnp.mean(d * d, axis=-1, keepdims=True)
    return d * lax.rsqrt(v + 1e-5)


def _gelu(x):
    u = x * (0.7978845608028654 + (0.7978845608028654 * 0.044715) * (x * x))
    hx = 0.5 * x
    return hx + hx * jnp.tanh(u)


def _dot(a, b):
    return jnp.dot(a, b, preferred_element_type=f32)


def _swap_cols(cols):
    chunk = lax.broadcasted_iota(jnp.int32, cols[0].shape, 1) // 4
    t = [pltpu.roll(v, 4 * g, 1) if g else v for g, v in enumerate(cols)]
    a = [t[-j % 8] for j in range(8)]
    for b in (1, 2, 4):
        hi = (chunk & b) != 0
        a = [jnp.where(hi, a[(j - b) % 8], a[j]) for j in range(8)]
    return [pltpu.roll(v, 128 - 4 * g, 1) if g else v for g, v in enumerate(a)]


def _swap_ref(ref, r0, rows, c0):
    cs = [pl.ds(c0 + g * 128, 128) for g in range(8)]
    cols = _swap_cols([pltpu.bitcast(ref[pl.ds(r0, rows), c], jnp.int32) for c in cs])
    for c, v in zip(cs, cols):
        ref[pl.ds(r0, rows), c] = pltpu.bitcast(v, bf16)


def _kernel(x_ref, c_ref, wmod_h, wqkv_h, wo_h, w1_h, w2_h, w3_h, w4_h, o_ref,
            wmod, wqkv, wo, w1, w2, w3, w4, mod, qkb, ob, xa, hb, gs, ub, scb, sems):
    i = pl.program_id(0)
    cps = [
        pltpu.make_async_copy(wmod_h.at[:, 0:2 * D], wmod.at[:, 0:2 * D], sems.at[0]),
        pltpu.make_async_copy(wmod_h.at[:, 2 * D:], wmod.at[:, 2 * D:], sems.at[1]),
        pltpu.make_async_copy(wo_h, wo, sems.at[2]),
        pltpu.make_async_copy(w1_h, w1, sems.at[3]),
        pltpu.make_async_copy(w2_h, w2, sems.at[4]),
        pltpu.make_async_copy(w3_h, w3, sems.at[5]),
        pltpu.make_async_copy(w4_h, w4, sems.at[6]),
    ]

    def qkv_copy(j):
        cs = pl.ds(pl.multiple_of(j * D, D), D)
        return pltpu.make_async_copy(wqkv_h.at[:, cs], wqkv.at[:, cs], sems.at[7 + j])

    def mrow(j):
        return mod[0:1, j * D:(j + 1) * D]

    def qkv():
        x = x_ref[...].astype(f32)
        h = (_ln(x) * (1.0 + mrow(1)) + mrow(0)).astype(bf16)
        ob[...] = h

        def body(j, carry):
            c0 = pl.multiple_of(j * D, D)

            @pl.when(i == 0)
            def _():
                qkv_copy(j).wait()

                def perm(r, carry2):
                    _swap_ref(wqkv, pl.multiple_of(r * 128, 128), 128, c0)
                    return carry2
                lax.fori_loop(0, D // 128, perm, 0)

            qkb[j, PAD:, :] = _dot(ob[...], wqkv[:, pl.ds(c0, D)])
            return carry
        lax.fori_loop(0, 3, body, 0)

    def attn(t, j):
        r0 = pl.multiple_of(j * R, R)
        css = [slice(g * 128, (g + 1) * 128) for g in range(8)]
        ps = [None] * W
        for cs in css:
            q = qkb[0, pl.ds(r0 + PAD, R), cs]
            k = qkb[1, pl.ds(r0, R + PAD), cs]
            for w in range(W):
                qk = q * k[PAD - DIL * w:PAD - DIL * w + R]
                ps[w] = qk if ps[w] is None else ps[w] + qk
        li = lax.broadcasted_iota(jnp.int32, (128, 128), 0) // 4
        lj = lax.broadcasted_iota(jnp.int32, (128, 128), 1) // 4
        p = (jnp.concatenate(ps, axis=0) * (DH ** -0.5)).astype(bf16)
        lg = _dot(p, (li == lj).astype(bf16))
        pos = t * T + r0 + lax.broadcasted_iota(jnp.int32, (R, 128), 0)
        ls = [lg[0:R]] + [jnp.where(pos >= DIL * w, lg[w * R:(w + 1) * R], -1e9)
                          for w in range(1, W)]
        m = ls[0]
        for l in ls[1:]:
            m = jnp.maximum(m, l)
        es = [jnp.exp(l - m) for l in ls]
        den = es[0]
        for e in es[1:]:
            den = den + e
        inv = 1.0 / den
        es = [e * inv for e in es]
        outs = []
        for cs in css:
            v = qkb[2, pl.ds(r0, R + PAD), cs]
            acc = None
            for w in range(W):
                pv = es[w] * v[PAD - DIL * w:PAD - DIL * w + R]
                acc = pv if acc is None else acc + pv
            outs.append(pltpu.bitcast(acc.astype(bf16), jnp.int32))
        for cs, o in zip(css, _swap_cols(outs)):
            ob[pl.ds(r0, R), cs] = pltpu.bitcast(o, bf16)

    def a_back(t):
        r0 = pl.multiple_of(t * T, T)
        qkb[1:3, 0:PAD, :] = qkb[1:3, T:T + PAD, :]
        x1 = x_ref[...].astype(f32) + mrow(2) * _dot(ob[...], wo[...])
        xa[pl.ds(r0, T), :] = x1
        h2 = _ln(x1) * (1.0 + mrow(4)) + mrow(3)
        hb[pl.ds(r0, T), :] = h2
        g1 = _gelu(_dot(_ln(h2).astype(bf16), w1[...]))
        gs[pl.ds(r0 + 8, T), :] = g1

    def b_front(t):
        r0 = pl.multiple_of(t * T, T)
        c = D // 4
        win = gs[pl.ds(r0, T + 16), :]
        gsh = jnp.concatenate([
            win[7:7 + T, 0:c], win[9:9 + T, c:2 * c],
            win[6:6 + T, 2 * c:3 * c], win[10:10 + T, 3 * c:]], axis=1).astype(bf16)
        x1 = hb[pl.ds(r0, T), :] + _dot(gsh, w2[...])
        hb[pl.ds(r0, T), :] = x1
        l = _ln(x1).astype(bf16)
        for j in range(F // FC):
            ub[:, j * FC:(j + 1) * FC] = _gelu(_dot(l, w3[:, j * FC:(j + 1) * FC])).astype(bf16)

    def w4_chunk(t, g):
        r0 = pl.multiple_of(t * T, T)
        cs = pl.ds(pl.multiple_of(g * 128, 128), 128)
        gb = mod[0:1, pl.ds(pl.multiple_of(5 * D + g * 128, 128), 128)]
        h2 = _dot(ub[...], w4[:, cs])
        o_ref[:, cs] = (xa[pl.ds(r0, T), cs] + gb * (hb[pl.ds(r0, T), cs] + h2)).astype(o_ref.dtype)

    def loop(*fns, U=2):
        def body(g, carry):
            for u in range(U):
                for fn, t in fns:
                    fn(t, g * U + u)
            return carry
        lax.fori_loop(0, D // 128 // U, body, 0)

    @pl.when(i == 0)
    def _():
        cps[0].start()
        for j in range(3):
            qkv_copy(j).start()
        for cp in cps[1:]:
            cp.start()
        qkb[1:3, 0:PAD, :] = jnp.zeros((2, PAD, D), f32)
        gs[0:8, :] = jnp.zeros((8, D), f32)
        gs[S + 8:, :] = jnp.zeros((8, D), f32)
        cv = c_ref[...].astype(f32)
        sc = jnp.broadcast_to(cv * jax.nn.sigmoid(cv), (16, D)).astype(bf16)
        cps[0].wait()
        mod[:, 0:2 * D] = _dot(sc, wmod[:, 0:2 * D])
        scb[...] = sc

    pl.when(i < NT)(qkv)
    pl.when(i < LAG)(lambda: loop((attn, i)))
    pl.when((i >= LAG) & (i < NT))(lambda: loop((attn, i), (w4_chunk, i - LAG), U=8))
    pl.when(i >= NT)(lambda: loop((w4_chunk, i - LAG), U=2))

    @pl.when(i == 0)
    def _():
        for cp in cps[1:4]:
            cp.wait()

        def body(j, carry):
            cs = pl.ds(pl.multiple_of(2 * D + j * 512, 512), 512)
            mod[:, cs] = _dot(scb[...], wmod[:, cs])
            return carry
        lax.fori_loop(0, 8, body, 0)

    pl.when(i < NT)(lambda: a_back(i))

    @pl.when(i == 1)
    def _():
        for cp in cps[4:6]:
            cp.wait()

    pl.when(i == LAG - 1)(cps[6].wait)
    pl.when((i >= 1) & (i <= NT))(lambda: b_front(i - 1))


@jax.jit
def pallas_adaLN_cond__sliding_local_dilated__mixer_s_mlp__prompt_kernel(
        A_x, A_wqkv, A_wo, B_x, B_w1, B_w2, B_w3, B_w4, c, w_mod):
    any_spec = pl.BlockSpec(memory_space=pl.ANY)
    ws = (w_mod, A_wqkv, A_wo, B_w1, B_w2, B_w3, B_w4)
    out = pl.pallas_call(
        _kernel,
        grid=(NT + LAG,),
        in_specs=[pl.BlockSpec((T, D), lambda i: (jnp.minimum(i, NT - 1), 0)),
                  pl.BlockSpec((1, D), lambda i: (0, 0))] + [any_spec] * 7,
        out_specs=pl.BlockSpec((T, D), lambda i: (jnp.maximum(i - LAG, 0), 0)),
        out_shape=jax.ShapeDtypeStruct((S, D), A_x.dtype),
        scratch_shapes=[pltpu.VMEM(w.shape, w.dtype) for w in ws] + [
            pltpu.VMEM((16, 6 * D), f32),
            pltpu.VMEM((3, T + PAD, D), f32),
            pltpu.VMEM((T, D), bf16),
            pltpu.VMEM((S, D), f32), pltpu.VMEM((S, D), f32),
            pltpu.VMEM((S + 16, D), f32),
            pltpu.VMEM((T, F), bf16),
            pltpu.VMEM((16, D), bf16),
            pltpu.SemaphoreType.DMA((10,)),
        ],
        compiler_params=pltpu.CompilerParams(
            dimension_semantics=("arbitrary",),
            vmem_limit_bytes=110 * 1024 * 1024),
    )(A_x.reshape(S, D), c, *ws)
    return out.reshape(A_x.shape)
```
